```python
import jax
import jax.numpy as jnp

def _softmax(x, axis=-1):
    return jax.nn.softmax(x, axis=axis)
def _gelu(x):
    return jax.nn.gelu(x, approximate=True)
def _silu(x):
    return jax.nn.silu(x)
def _sigmoid(x):
    return jax.nn.sigmoid(x)
def _layernorm(x, axis=-1, eps=1e-5):
    m = jnp.mean(x, axis=axis, keepdims=True)
    v = jnp.var(x, axis=axis, keepdims=True)
    return (x - m) / jnp.sqrt(v + eps)
def _scatter_add(tgt, idx, src, axis=0):
    return tgt.at[idx].add(src)
def _segment_sum(src, seg, n):
    return jax.ops.segment_sum(src, seg, n)
class _Rng:
    def __init__(self, key):
        self._k = key
    def _next(self):
        self._k, sub = jax.random.split(self._k)
        return sub
    def normal(self, shape):
        return jax.random.normal(self._next(), shape, dtype=jnp.bfloat16)
    def randint(self, lo, hi, shape):
        return jax.random.randint(self._next(), shape, lo, hi, dtype=jnp.int32)
    def uniform(self, shape, lo=0.0, hi=1.0):
        return jax.random.uniform(self._next(), shape, jnp.bfloat16, lo, hi)
    def permutation(self, n):
        return jax.random.permutation(self._next(), n)


kernel_name = 'concat_heads__compressed_kv_cla__gqa_block_cached__decode'

def setup_inputs():
    _rng = _Rng(jax.random.key(int.from_bytes(__import__("os").urandom(4), "little")))
    _w = (lambda a: (lambda t: t.astype(jnp.bfloat16) if jnp.issubdtype(t.dtype, jnp.floating) else t)(jnp.asarray(a)))
    def _A_setup():
        B, H, Sq, Sk, D, M = 2, 32, 1, 4096, 128, 512
        Dc = 4 * D
        return {
            "x": _w((lambda *s: _rng.normal(s) * 0.05)(B, Sq, M)),
            "c_kv": _w((lambda *s: _rng.normal(s) * 0.05)(B, Sk, Dc)),
            "w_q": _w((lambda *s: _rng.normal(s) * 0.05)(M, H, D) * (M ** -0.5)),
            "w_uk": _w((lambda *s: _rng.normal(s) * 0.05)(Dc, H, D) * (Dc ** -0.5)),
            "w_uv": _w((lambda *s: _rng.normal(s) * 0.05)(Dc, H, D) * (Dc ** -0.5)),
            "w_o": _w((lambda *s: _rng.normal(s) * 0.05)(H, D, M) * ((H * D) ** -0.5)),
        }
    _A_in = _A_setup()

    def _B_setup():
        B, Sq, D = 2, 1, 512
        Hq, Hkv, Sk, Dh = 32, 32, 4096, 128
        assert Hq % Hkv == 0, (Hq, Hkv)
        return {
            "x": _w((lambda *s: _rng.normal(s) * 0.05)(B, Sq, D)),
            "k_cache": _w((lambda *s: _rng.normal(s) * 0.05)(B, Hkv, Sk, Dh)),
            "v_cache": _w((lambda *s: _rng.normal(s) * 0.05)(B, Hkv, Sk, Dh)),
            "wq": _w((lambda *s: _rng.normal(s) * 0.05)(D, Hq * Dh) * (D ** -0.5)),
            "wo": _w((lambda *s: _rng.normal(s) * 0.05)(Hq * Dh, D) * ((Hq * Dh) ** -0.5)),
        }
    _B_in = _B_setup()

    return {
        "A_x": _A_in["x"],
        "A_c_kv": _A_in["c_kv"],
        "A_w_q": _A_in["w_q"],
        "A_w_uk": _A_in["w_uk"],
        "A_w_uv": _A_in["w_uv"],
        "A_w_o": _A_in["w_o"],
        "B_x": _B_in["x"],
        "B_k_cache": _B_in["k_cache"],
        "B_v_cache": _B_in["v_cache"],
        "B_wq": _B_in["wq"],
        "B_wo": _B_in["wo"],
    }

def reference(A_x, A_c_kv, A_w_q, A_w_uk, A_w_uv, A_w_o, B_x, B_k_cache, B_v_cache, B_wq, B_wo):
    def _A_ref(x, c_kv, w_q, w_uk, w_uv, w_o):
        B, Sq, M = x.shape[0], x.shape[1], x.shape[2]
        Sk = c_kv.shape[1]
        H, D = w_q.shape[1], w_q.shape[2]
        q = jnp.einsum("bqm,mhd->bhqd", x, w_q)
        k = jnp.einsum("bkc,chd->bhkd", c_kv, w_uk)
        v = jnp.einsum("bkc,chd->bhkd", c_kv, w_uv)
        scores = jnp.einsum("bhqd,bhkd->bhqk", q, k) * (D ** -0.5)
        off = Sk - Sq
        qi = jnp.arange(Sq)[:, None]
        kj = jnp.arange(Sk)[None, :]
        cmask = kj <= (qi + off)
        scores = jnp.where(cmask[None, None], scores, -1e9)
        p = _softmax(scores, axis=-1)
        ctx = jnp.einsum("bhqk,bhkd->bhqd", p, v)
        return jnp.einsum("bhqd,hdm->bqm", ctx, w_o)

    def _B_ref(x, k_cache, v_cache, wq, wo):
        B, Sq, D = x.shape
        Hq, Dh = 32, 128
        Hkv = k_cache.shape[1]
        rep = Hq // Hkv
        q = (lambda x, *d: x.transpose(*d))((x @ wq).reshape(B, Sq, Hq, Dh), 0, 2, 1, 3)
        k = jnp.repeat(k_cache, rep, axis=1)
        v = jnp.repeat(v_cache, rep, axis=1)
        scores = jnp.einsum("bhqd,bhkd->bhqk", q, k) * (Dh ** -0.5)
        p = _softmax(scores, axis=-1)
        o = jnp.einsum("bhqk,bhkd->bhqd", p, v)
        return (lambda x, *d: x.transpose(*d))(o, 0, 2, 1, 3).reshape(B, Sq, Hq * Dh) @ wo

    a = _A_ref(A_x, A_c_kv, A_w_q, A_w_uk, A_w_uv, A_w_o)
    b = _B_ref(B_x, B_k_cache, B_v_cache, B_wq, B_wo)
    return jnp.concatenate([a, b], axis=-1)
```

```python
import functools
import jax
import jax.numpy as jnp
from jax.experimental import pallas as pl
from jax.experimental.pallas import tpu as pltpu

F32 = jnp.float32
BF16 = jnp.bfloat16
NT = (((1,), (1,)), ((), ()))

B, H, S, D, M, C = 2, 32, 4096, 128, 512, 512
NSLOT = 3
TILE = 128


def _kernel(xa_hbm, c_hbm, wqa_hbm, wuk_hbm, wuv_hbm, woa_hbm, xb_hbm, k_hbm, v_hbm, wqb_hbm, wob_hbm,
            out_ref,
            xa_v, xb_v, c_v, wqa_v, wuk_v, wuv_v, woa_v, wqb_v, wob_v, k_v, v_v,
            qb_s, ob_s, oa_s, qabs_s, ctx_s, s_s,
            sem_x, sem_w, sem_k, sem_v, sem_o):
    def rows(src, dst, sem, n, r0=0, r1=None):
        r1 = src.shape[0] if r1 is None else r1
        return [pltpu.make_async_copy(src.at[pl.ds(r, n)], dst.at[pl.ds(r, n)], sem) for r in range(r0, r1, n)]

    def wqb_descs(sem):
        return [pltpu.make_async_copy(wqb_hbm.at[pl.ds(r, 16), pl.ds(c, 1024)], wqb_v.at[pl.ds(r, 16), pl.ds(c, 1024)], sem)
                for r in range(0, M, 16) for c in range(0, H * D, 1024)]

    def kv_descs(i, slot):
        out = []
        for t in range(S // TILE):
            src = pl.ds(pl.multiple_of(i * S + t * TILE, TILE), TILE)
            dst = pl.ds(t * TILE, TILE)
            out.append((pltpu.make_async_copy(k_hbm.at[src], k_v.at[slot, dst], sem_k.at[slot]),
                        pltpu.make_async_copy(v_hbm.at[src], v_v.at[slot, dst], sem_v.at[slot])))
        return out

    def wait_all(buf, sem):
        pltpu.make_async_copy(buf, buf, sem).wait()

    class Stream:
        def __init__(self, pairs):
            self.pairs, self.pos = pairs, 0
        def issue(self, n):
            for a, b in self.pairs[self.pos:self.pos + n]:
                a.start(priority=0)
                b.start(priority=1)
            self.pos = min(self.pos + n, len(self.pairs))
        def flush(self):
            self.issue(len(self.pairs) - self.pos)

    NWO = 8
    wo_rows = H * D // NWO
    pre = (list(zip(rows(wqa_hbm, wqa_v, sem_w.at[0], TILE), rows(wuk_hbm, wuk_v, sem_w.at[1], TILE)))
           + list(zip(rows(c_hbm, c_v, sem_w.at[2], 32, 0, S), rows(c_hbm, c_v, sem_w.at[3], 32, S, 2 * S)))
           + list(zip(wqb_descs(sem_w.at[4]), rows(wuv_hbm, wuv_v, sem_w.at[5], TILE)))
           + kv_descs(0, 0) + kv_descs(1, 1))
    st = Stream(pre)
    post = []
    for g in range(NWO):
        post += list(zip(rows(woa_hbm, woa_v, sem_o.at[0, g], 32, g * wo_rows, (g + 1) * wo_rows),
                         rows(wob_hbm, wob_v, sem_o.at[1, g], 32, g * wo_rows, (g + 1) * wo_rows)))

    cxa = pltpu.make_async_copy(xa_hbm, xa_v, sem_x.at[0])
    cxb = pltpu.make_async_copy(xb_hbm, xb_v, sem_x.at[1])
    st.issue(4)
    cxa.start()
    cxb.start()
    st.issue(128 - 4 + 32)
    cxa.wait()
    cxb.wait()

    def rep16(x_v):
        return jnp.concatenate([jnp.broadcast_to(x_v[pl.ds(b, 1), :].astype(F32), (8, M)) for b in range(B)], axis=0).astype(BF16)

    def head_pair(w_v, j):
        w = w_v.bitcast(jnp.uint32)[pl.ds(j, M, stride=H // 2), :]
        lo = pltpu.bitcast(w << 16, F32).astype(BF16)
        hi = pltpu.bitcast(w & jnp.uint32(0xFFFF0000), F32).astype(BF16)
        return lo, hi

    xa = rep16(xa_v)
    wait_all(wqa_v, sem_w.at[0])
    wait_all(wuk_v, sem_w.at[1])
    for j in range(H // 2):
        wq2 = head_pair(wqa_v, j)
        wk2 = head_pair(wuk_v, j)
        for e in range(2):
            h = 2 * j + e
            q = jnp.dot(xa, wq2[e], preferred_element_type=F32).astype(BF16)
            qa = lax_dot_nt(q, wk2[e])
            for b in range(B):
                qabs_s[b, pl.ds(h, 1), :] = qa[8 * b:8 * b + 1, :]
        st.issue(6)
    scale = D ** -0.5
    CH = 512
    for b in range(B):
        wait_all(c_v.at[pl.ds(b * S, S)], sem_w.at[2 + b])
    for b in range(B):
        qa = qabs_s[b].astype(BF16)
        for t in range(S // CH):
            s_s[:, t * CH:(t + 1) * CH] = lax_dot_nt(qa, c_v[pl.ds(b * S + t * CH, CH), :])
            st.issue(4)
        s = s_s[...]
        m = jnp.max(s, axis=-1, keepdims=True)
        p = jnp.exp((s - m) * scale)
        l = jnp.sum(p, axis=-1, keepdims=True)
        pb = p.astype(BF16)
        acc = jnp.zeros((H, C), F32)
        for t in range(S // CH):
            acc += jnp.dot(pb[:, t * CH:(t + 1) * CH], c_v[pl.ds(b * S + t * CH, CH), :], preferred_element_type=F32)
            st.issue(4)
        ctx_s[b] = acc / l
    xb = rep16(xb_v)
    wait_all(wqb_v, sem_w.at[4])
    for g in range(8):
        q = jnp.dot(xb, wqb_v[:, g * 512:(g + 1) * 512], preferred_element_type=F32)
        for u in range(4):
            for b in range(B):
                qb_s[b * H + g * 4 + u] = q[8 * b:8 * b + 8, u * D:(u + 1) * D]
        st.issue(2)
    wait_all(wuv_v, sem_w.at[5])
    for j in range(H // 2):
        wv2 = head_pair(wuv_v, j)
        for e in range(2):
            h = 2 * j + e
            lhs = jnp.concatenate([jnp.broadcast_to(ctx_s[b, pl.ds(h, 1), :], (8, C)) for b in range(B)], axis=0)
            oa_s[h] = jnp.dot(lhs.astype(BF16), wv2[e], preferred_element_type=F32)
        st.issue(1)
    st.flush()

    NCH = 4
    CK = S // NCH

    def head(i, slot, stream):
        per = len(stream.pairs) // (2 * NCH)
        q = qb_s[i].astype(BF16)
        wait_all(k_v.at[slot], sem_k.at[slot])
        ss = []
        for t in range(NCH):
            stream.issue(per)
            ss.append(lax_dot_nt(q, k_v[slot, pl.ds(t * CK, CK), :]))
        s = jnp.concatenate(ss, axis=-1)
        m = jnp.max(s, axis=-1, keepdims=True)
        p = jnp.exp((s - m) * scale)
        l = jnp.sum(p, axis=-1, keepdims=True)
        pb = p.astype(BF16)
        wait_all(v_v.at[slot], sem_v.at[slot])
        acc = jnp.zeros((8, D), F32)
        for t in range(NCH):
            stream.issue(per)
            acc += jnp.dot(pb[:, t * CK:(t + 1) * CK], v_v[slot, pl.ds(t * CK, CK), :], preferred_element_type=F32)
        stream.flush()
        return acc / l

    def store_o(i, o):
        b = i // H
        h = i % H
        ob_s[h, pl.ds(pl.multiple_of(b * 8, 8), 8), :] = o

    def body(i, _):
        slot = i % NSLOT
        o = head(i, slot, Stream(kv_descs(i + 2, (i + 2) % NSLOT)))
        store_o(i, o)
        return 0

    NH = B * H
    jax.lax.fori_loop(0, NH - 2, body, 0)
    half = len(post) // 2
    for n, i in enumerate(range(NH - 2, NH)):
        o = head(i, i % NSLOT, Stream(post[n * half // 2:(n + 1) * half // 2]))
        ob_s[i % H, pl.ds((i // H) * 8, 8), :] = o
    st = Stream(post[half:])

    acc_a = jnp.zeros((16, M), F32)
    acc_b = jnp.zeros((16, M), F32)
    hg = H // NWO
    for g in range(NWO):
        st.issue(16)
        la = jnp.concatenate([oa_s[g * hg + u] for u in range(hg)], axis=-1).astype(BF16)
        lb = jnp.concatenate([ob_s[g * hg + u] for u in range(hg)], axis=-1).astype(BF16)
        wait_all(woa_v.at[pl.ds(g * wo_rows, wo_rows)], sem_o.at[0, g])
        acc_a += jnp.dot(la, woa_v[pl.ds(g * wo_rows, wo_rows), :], preferred_element_type=F32)
        wait_all(wob_v.at[pl.ds(g * wo_rows, wo_rows)], sem_o.at[1, g])
        acc_b += jnp.dot(lb, wob_v[pl.ds(g * wo_rows, wo_rows), :], preferred_element_type=F32)
    for b in range(B):
        out_ref[pl.ds(b, 1), 0:M] = acc_a[8 * b:8 * b + 1, :].astype(out_ref.dtype)
        out_ref[pl.ds(b, 1), M:2 * M] = acc_b[8 * b:8 * b + 1, :].astype(out_ref.dtype)


def lax_dot_nt(a, b):
    return jax.lax.dot_general(a, b, NT, preferred_element_type=F32)


@jax.jit
def pallas_concat_heads__compressed_kv_cla__gqa_block_cached__decode_kernel(
        A_x, A_c_kv, A_w_q, A_w_uk, A_w_uv, A_w_o, B_x, B_k_cache, B_v_cache, B_wq, B_wo):
    any_spec = pl.BlockSpec(memory_space=pl.ANY)
    vm = pltpu.VMEM
    return pl.pallas_call(
        _kernel,
        in_specs=[any_spec] * 11,
        out_specs=pl.BlockSpec(memory_space=pltpu.VMEM),
        out_shape=jax.ShapeDtypeStruct((B, 2 * M), A_x.dtype),
        scratch_shapes=[
            vm((B, M), BF16), vm((B, M), BF16),
            vm((B * S, C), BF16),
            vm((M * H, D), BF16), vm((C * H, D), BF16), vm((C * H, D), BF16),
            vm((H * D, M), BF16), vm((M, H * D), BF16), vm((H * D, M), BF16),
            vm((NSLOT, S, D), BF16), vm((NSLOT, S, D), BF16),
            vm((B * H, 8, D), F32), vm((H, 16, D), F32), vm((H, 16, D), F32),
            vm((B, H, C), F32), vm((B, H, C), F32), vm((H, S), F32),
            pltpu.SemaphoreType.DMA((2,)), pltpu.SemaphoreType.DMA((6,)),
            pltpu.SemaphoreType.DMA((NSLOT,)), pltpu.SemaphoreType.DMA((NSLOT,)),
            pltpu.SemaphoreType.DMA((2, 8)),
        ],
        compiler_params=pltpu.CompilerParams(vmem_limit_bytes=64 << 20),
    )(A_x.reshape(B, M), A_c_kv.reshape(B * S, C), A_w_q.reshape(M * H, D), A_w_uk.reshape(C * H, D), A_w_uv.reshape(C * H, D),
      A_w_o.reshape(H * D, M), B_x.reshape(B, M), B_k_cache.reshape(B * H * S, D), B_v_cache.reshape(B * H * S, D), B_wq, B_wo).reshape(B, 1, 2 * M)
```

```python
import jax
import jax.numpy as jnp
from jax import lax
from jax.experimental import pallas as pl
from jax.experimental.pallas import tpu as pltpu

F32 = jnp.float32
BF16 = jnp.bfloat16

B, H, S, D, M, C = 2, 32, 4096, 128, 512, 512
NH = B * H
DESC = 16384
UNIT = S * D // DESC
WP = M * H * D // DESC
CH = 512


def _dot(a, b):
    return jnp.dot(a, b, preferred_element_type=F32)


def _dot_nt(a, b):
    return lax.dot_general(a, b, (((1,), (1,)), ((), ())), preferred_element_type=F32)


def _fold(x, op):
    parts = [x[:, c:c + 128] for c in range(0, x.shape[1], 128)]
    while len(parts) > 1:
        parts = [op(parts[i], parts[i + 1]) for i in range(0, len(parts), 2)]
    return parts[0]


def make(N0=160, N1=10, N2=5, N3=8, N4=30, NSLOT=8, WO_GROUPS=(12, 10, 6, 3, 1), nobounds=False, scopes=False,
         hsplit=2, xfirst=True):
    NWO = len(WO_GROUPS)
    assert sum(WO_GROUPS) == H
    NC = S // CH
    G1 = N0
    G2 = G1 + N1 * H // 2
    G3 = G2 + N2 * 2 * B * NC
    G4 = G3 + N3 * H // 2
    G5 = G4 + N4 * NH
    OFF_C, OFF_WQV, OFF_KV = WP, 2 * WP, 3 * WP
    OFF_WO = OFF_KV + NH * UNIT
    END = OFF_WO + WP
    assert G1 >= OFF_C and G2 >= OFF_WQV and G3 >= OFF_KV
    assert G4 <= OFF_KV + NSLOT * UNIT
    for i in range(NH):
        assert G4 + N4 * i >= OFF_KV + UNIT * (i + 1)
        assert min(G4 + N4 * (i + 1), OFF_WO) <= OFF_KV + UNIT * (i + NSLOT)
    import contextlib
    scope = (lambda n: jax.named_scope(n)) if scopes else (lambda n: contextlib.nullcontext())

    def _kernel(xa_hbm, c_hbm, wqa_hbm, wuk_hbm, wuv_hbm, woa_hbm, xb_hbm, k_hbm, v_hbm, wqb_hbm, wob_hbm,
                out_ref,
                xa_v, xb_v, c_v, wqa_v, wuk_v, wuv_v, woa_v, wqb_v, wob_v, k_v, v_v,
                qb_s, oa_s, ob_s, qabs_s, ctx_s, s_s,
                sem_x, sem_w, sem_k, sem_v, sem_o):
        scale = D ** -0.5

        def rows(src, dst, sem, t, td=None):
            n = DESC // src.shape[1]
            td = t if td is None else td
            return pltpu.make_async_copy(src.at[pl.ds(pl.multiple_of(t * n, n), n)],
                                         dst.at[pl.ds(pl.multiple_of(td * n, n), n)], sem)

        def wait(buf, sem):
            pltpu.make_async_copy(buf, buf, sem).wait()

        def pair_wqk(t):
            return rows(wqa_hbm, wqa_v, sem_w.at[0], t), rows(wuk_hbm, wuk_v, sem_w.at[1], t)

        def pair_c(t):
            return rows(c_hbm, c_v, sem_w.at[2], t), rows(c_hbm, c_v, sem_w.at[3], t + WP)

        def pair_wqv(t):
            r = pl.ds(pl.multiple_of((t >> 1) * 8, 8), 8)
            c = pl.ds(pl.multiple_of((t & 1) * (DESC // 8), DESC // 8), DESC // 8)
            return (pltpu.make_async_copy(wqb_hbm.at[r, c], wqb_v.at[r, c], sem_w.at[4]),
                    rows(wuv_hbm, wuv_v, sem_w.at[5], t))

        def pair_kv(t):
            td = lax.rem(t, NSLOT * UNIT)
            slot = lax.div(td, UNIT)
            return rows(k_hbm, k_v, sem_k.at[slot], t, td), rows(v_hbm, v_v, sem_v.at[slot], t, td)

        def pair_wo(g):
            return lambda t: (rows(woa_hbm, woa_v, sem_o.at[0, g], t), rows(wob_hbm, wob_v, sem_o.at[1, g], t))

        segments = [(0, OFF_C, 0, pair_wqk), (OFF_C, OFF_WQV, OFF_C, pair_c), (OFF_WQV, OFF_KV, OFF_WQV, pair_wqv),
                    (OFF_KV, OFF_WO, OFF_KV, pair_kv)]
        h0 = 0
        for g, nh in enumerate(WO_GROUPS):
            segments.append((OFF_WO + h0 * WP // H, OFF_WO + (h0 + nh) * WP // H, OFF_WO, pair_wo(g)))
            h0 += nh

        def issue(g0, n, lo, hi):
            static = isinstance(g0, int)
            for s0, s1, base, pair in segments:
                if s1 <= lo or hi <= s0:
                    continue

                def one(t, carry, pair=pair):
                    a, b = pair(t)
                    a.start(priority=0)
                    b.start(priority=1)
                    return carry
                if static:
                    first, last = max(g0, s0), min(g0 + n, s1)
                else:
                    first = g0 if s0 <= lo else jnp.maximum(g0, s0)
                    last = g0 + n if hi <= s1 else jnp.minimum(g0 + n, s1)
                lax.fori_loop(first - base, last - base, one, 0)

        copy_xa = pltpu.make_async_copy(xa_hbm, xa_v, sem_x.at[0])
        copy_xb = pltpu.make_async_copy(xb_hbm, xb_v, sem_x.at[1])
        with scope("p0"):
            if xfirst:
                copy_xa.start()
                copy_xb.start(priority=1)
                issue(0, G1, 0, G1)
            else:
                issue(0, 8, 0, 8)
                copy_xa.start()
                copy_xb.start(priority=1)
                issue(8, G1 - 8, 8, G1)
            copy_xa.wait()
            copy_xb.wait()

        def rep_rows(row):
            return jnp.concatenate([jnp.broadcast_to(row(b).astype(F32), (8, M)) for b in range(B)], axis=0).astype(BF16)

        def head_pair(w_v, jj, u):
            w32 = w_v.bitcast(jnp.uint32).at[pl.ds(pl.multiple_of(jj * 4, 4), M * H // 2 - 12)]
            w = w32[pl.ds(u, M, stride=H // 2), :]
            lo = pltpu.bitcast(w << 16, F32).astype(BF16)
            hi = pltpu.bitcast(w & jnp.uint32(0xFFFF0000), F32).astype(BF16)
            return lo, hi

        wait(wqa_v, sem_w.at[0])
        wait(wuk_v, sem_w.at[1])
        xa = rep_rows(lambda b: xa_v[pl.ds(b, 1), :])

        def absorb(jj, carry):
            for u in range(4):
                issue(G1 + (jj * 4 + u) * N1, N1, G1, G2)
                wq2 = head_pair(wqa_v, jj, u)
                wk2 = head_pair(wuk_v, jj, u)
                for e in range(2):
                    q = _dot(xa, wq2[e]).astype(BF16)
                    qa = _dot_nt(q, wk2[e])
                    for b in range(B):
                        qabs_s[b, jj, pl.ds(2 * u + e, 1), :] = qa[8 * b:8 * b + 1, :]
            return carry

        with scope("p1"):
            lax.fori_loop(0, H // 8, absorb, 0)

        wait(c_v.at[pl.ds(0, S)], sem_w.at[2])
        wait(c_v.at[pl.ds(S, S)], sem_w.at[3])

        def latent(b, carry):
            qa = qabs_s[b].reshape(H, C).astype(BF16)

            def chunk(t):
                return c_v[pl.ds(pl.multiple_of(b * S + t * CH, CH), CH), :]

            def scores(t, m):
                issue(G2 + (2 * b * NC + t) * N2, N2, G2, G3)
                s = _dot_nt(qa, chunk(t))
                s_s[t] = s
                return jnp.maximum(m, _fold(s, jnp.maximum))

            m = lax.fori_loop(0, NC, scores, jnp.full((H, 128), -jnp.inf, F32))
            m = jnp.max(m, axis=-1, keepdims=True)

            def values(t, carry):
                l, acc = carry
                issue(G2 + ((2 * b + 1) * NC + t) * N2, N2, G2, G3)
                p = jnp.exp((s_s[t] - m) * scale)
                return l + _fold(p, jnp.add), acc + _dot(p.astype(BF16), chunk(t))

            l, acc = lax.fori_loop(0, NC, values, (jnp.zeros((H, 128), F32), jnp.zeros((H, C), F32)))
            ctx_s[b] = (acc / jnp.sum(l, axis=-1, keepdims=True)).reshape(H // 8, 8, C)
            return carry

        with scope("p2"):
            lax.fori_loop(0, B, latent, 0)

        wait(wqb_v, sem_w.at[4])
        wait(wuv_v, sem_w.at[5])
        xb = rep_rows(lambda b: xb_v[pl.ds(b, 1), :])

        def project(jj, carry):
            for u in range(4):
                j = jj * 4 + u
                issue(G3 + j * N3, N3, G3, G4)
                q = _dot(xb, wqb_v[:, pl.ds(pl.multiple_of(j * 2 * D, 2 * D), 2 * D)])
                wv2 = head_pair(wuv_v, jj, u)
                for e in range(2):
                    h = 2 * j + e
                    for b in range(B):
                        qb_s[b * H + h] = q[8 * b:8 * b + 8, e * D:(e + 1) * D]
                    oa_s[h] = _dot(rep_rows(lambda b: ctx_s[b, jj, pl.ds(2 * u + e, 1), :]), wv2[e])
            return carry

        with scope("p3"):
            lax.fori_loop(0, H // 8, project, 0)

        def head(i, carry):
            slot = lax.rem(i, NSLOT)
            r = pl.ds(pl.multiple_of(slot * S, S), S)
            n_a = N4 // 2 if hsplit == 2 else N4
            q = qb_s[i].astype(BF16)
            issue(G4 + i * N4, n_a, G4, G5)
            wait(k_v.at[r], sem_k.at[slot])
            s = _dot_nt(q, k_v[r, :])
            m = jnp.max(_fold(s, jnp.maximum), axis=-1, keepdims=True)
            p = jnp.exp((s - m) * scale)
            l = jnp.sum(_fold(p, jnp.add), axis=-1, keepdims=True)
            if hsplit == 2:
                issue(G4 + i * N4 + n_a, N4 - n_a, G4, G5)
            wait(v_v.at[r], sem_v.at[slot])
            o = _dot(p.astype(BF16), v_v[r, :]) / l
            ob_s[lax.rem(i, H), pl.ds(pl.multiple_of(lax.div(i, H) * 8, 8), 8), :] = o
            return carry

        with scope("p4"):
            lax.fori_loop(0, NH, head, 0)

        with scope("p5"):
            if G5 < END:
                issue(G5, END - G5, G5, END)
            accs = [jnp.zeros((8 * B, M), F32)] * 2
            h0 = 0
            for g, nh in enumerate(WO_GROUPS):
                r = pl.ds(h0 * D, nh * D)
                for side, (o_s, w_v) in enumerate(((oa_s, woa_v), (ob_s, wob_v))):
                    lhs = jnp.concatenate([o_s[h0 + u] for u in range(nh)], axis=-1).astype(BF16)
                    wait(w_v.at[r], sem_o.at[side, g])
                    accs[side] = accs[side] + _dot(lhs, w_v[r, :])
                h0 += nh
            for b in range(B):
                for side in range(2):
                    out_ref[pl.ds(b, 1), side * M:(side + 1) * M] = accs[side][8 * b:8 * b + 1, :].astype(out_ref.dtype)

    def fn(A_x, A_c_kv, A_w_q, A_w_uk, A_w_uv, A_w_o, B_x, B_k_cache, B_v_cache, B_wq, B_wo):
        vm = pltpu.VMEM
        out = pl.pallas_call(
            _kernel,
            in_specs=[pl.BlockSpec(memory_space=pl.ANY)] * 11,
            out_specs=pl.BlockSpec(memory_space=pltpu.VMEM),
            out_shape=jax.ShapeDtypeStruct((B, 2 * M), A_x.dtype),
            scratch_shapes=[
                vm((B, M), BF16), vm((B, M), BF16),
                vm((B * S, C), BF16),
                vm((M * H, D), BF16), vm((C * H, D), BF16), vm((C * H, D), BF16),
                vm((H * D, M), BF16), vm((M, H * D), BF16), vm((H * D, M), BF16),
                vm((NSLOT * S, D), BF16), vm((NSLOT * S, D), BF16),
                vm((NH, 8, D), F32), vm((H, 8 * B, D), F32), vm((H, 8 * B, D), F32),
                vm((B, H // 8, 8, C), F32), vm((B, H // 8, 8, C), F32), vm((S // CH, H, CH), F32),
                pltpu.SemaphoreType.DMA((2,)), pltpu.SemaphoreType.DMA((6,)),
                pltpu.SemaphoreType.DMA((NSLOT,)), pltpu.SemaphoreType.DMA((NSLOT,)),
                pltpu.SemaphoreType.DMA((2, NWO)),
            ],
            compiler_params=pltpu.CompilerParams(vmem_limit_bytes=100 << 20, disable_bounds_checks=nobounds),
        )(A_x.reshape(B, M), A_c_kv.reshape(B * S, C),
          A_w_q.reshape(M * H, D), A_w_uk.reshape(C * H, D), A_w_uv.reshape(C * H, D), A_w_o.reshape(H * D, M),
          B_x.reshape(B, M), B_k_cache.reshape(NH * S, D), B_v_cache.reshape(NH * S, D), B_wq, B_wo)
        return out.reshape(B, 1, 2 * M)
    return fn


_impl = make(nobounds=True)


@jax.jit
def pallas_concat_heads__compressed_kv_cla__gqa_block_cached__decode_kernel(
        A_x, A_c_kv, A_w_q, A_w_uk, A_w_uv, A_w_o, B_x, B_k_cache, B_v_cache, B_wq, B_wo):
    return _impl(A_x, A_c_kv, A_w_q, A_w_uk, A_w_uv, A_w_o, B_x, B_k_cache, B_v_cache, B_wq, B_wo)
```

```python
import contextlib
import functools
import jax
import jax.numpy as jnp
from jax import lax
from jax.experimental import pallas as pl
from jax.experimental.pallas import tpu as pltpu

F32 = jnp.float32
BF16 = jnp.bfloat16

B, H, S, D, M, C = 2, 32, 4096, 128, 512, 512
NH = B * H
DESC = 16384
PER_HEAD = S * D // DESC
PER_W = M * H * D // DESC


def _dot(a, b):
    return jnp.dot(a, b, preferred_element_type=F32)


def _dot_nt(a, b):
    return lax.dot_general(a, b, (((1,), (1,)), ((), ())), preferred_element_type=F32)


def _fold(x, op):
    parts = [x[:, c:c + 128] for c in range(0, x.shape[1], 128)]
    while len(parts) > 1:
        parts = [op(parts[i], parts[i + 1]) for i in range(0, len(parts), 2)]
    return parts[0]


def make(X0=24, N1=5, N2=5, N3=6, N5=21, N6=0, VX=0, WOB=(4, 2, 1, 1), LA=6, nobounds=False, nosem=False, scopes=False, SHIFT=1, WNS=8,
         CH=512, hsplit=2, WOA_NS=1, vmem=80):
    NC = S // CH
    NSTR = 4
    NSLOT = 3
    NSB = NH // NSTR
    WF = PER_W - SHIFT
    KF = PER_HEAD - SHIFT
    OFF_C, OFF_QV, OFF_KV = WF, 2 * WF, 3 * WF
    END_A = OFF_KV + LA * KF
    G1 = WF + X0
    G2 = G1 + N1 * 32
    G3 = G2 + N2 * 2 * B * NC
    G4 = G3 + N3 * 16
    assert G2 >= OFF_QV and G3 >= OFF_KV and G4 >= END_A and NSTR <= LA <= 2 * NSTR
    QR = H * D // 4
    G5 = LA * N5
    assert G5 >= 2 * KF and G5 + 8 * N6 >= 4 * KF
    SEM_QK, SEM_C, SEM_QV, SEM_WOA, SEM_WOB = 3, 4, 2, 1, 2
    NSEM = max(5, SEM_WOB + len(WOB))
    assert sum(WOB) == 8 and (NSB - 1) % NSLOT == 0
    scope = (lambda n: jax.named_scope(n)) if scopes else (lambda n: contextlib.nullcontext())

    def _kernel(xa_hbm, c_hbm, wqa_hbm, wuk_hbm, wuv_hbm, woa_hbm, xb_hbm, k_hbm, v_hbm, wqb_hbm, wob_hbm,
                out_ref,
                xa_v, xb_v, c_v, wqa_v, wuk_v, wuv_v, wqb_v, wo_v, k_v, v_v,
                xa_s, qb_s, o_s, qabs_s, ctx_s, s_s, sems):
        scale = D ** -0.5

        def whole(src, dst, sem, c, src0=0, dst0=0):
            n = DESC // src.shape[1]
            off = c * n + SHIFT * (n // 2)
            return pltpu.make_async_copy(src.at[pl.ds(pl.multiple_of(src0 + off, n // 2), n)],
                                         dst.at[pl.ds(pl.multiple_of(dst0 + off, n // 2), n)], sems.at[sem])

        def edge(src, dst, sem, e, count, src0=0, dst0=0):
            n = DESC // src.shape[1]
            off = e * (count * n - n // 2)
            return pltpu.make_async_copy(src.at[pl.ds(pl.multiple_of(src0 + off, n // 2), n // 2)],
                                         dst.at[pl.ds(pl.multiple_of(dst0 + off, n // 2), n // 2)], sems.at[sem])

        def spread(t, count, streams):
            if streams == 1:
                return t
            return (t & (streams - 1)) * (count // streams) + (t >> (streams.bit_length() - 1))

        def start(pair):
            pair[0].start(priority=0)
            pair[1].start(priority=1)

        def wait(buf, sem):
            pltpu.make_async_copy(buf, buf, sems.at[sem]).wait()

        def wqb_piece(c, col, width):
            r = pl.ds(pl.multiple_of((c >> 1) * 8, 8), 8)
            cols = pl.ds(pl.multiple_of((c & 1) * (DESC // 8) + col, width), width)
            return pltpu.make_async_copy(wqb_hbm.at[r, cols], wqb_v.at[r, cols], sems.at[SEM_QV])

        def pair_qk(t):
            c = spread(t, PER_W, WNS)
            return whole(wqa_hbm, wqa_v, SEM_QK, c), whole(wuk_hbm, wuk_v, SEM_QK, c)

        def pair_c(t):
            c = spread(t, PER_W, WNS)
            return whole(c_hbm, c_v, SEM_C, c), whole(c_hbm, c_v, SEM_C, c, S, S)

        def pair_qv(t):
            c = spread(t, PER_W, WNS)
            return wqb_piece(c, 0, DESC // 8), whole(wuv_hbm, wuv_v, SEM_QV, c)

        def kv_rows(g, j):
            slot = lax.rem(g, NSLOT)
            return slot, (j * NSB + g) * S, (slot * NSTR + j) * S

        def pair_kv(g, t):
            slot, src0, dst0 = kv_rows(g, t & (NSTR - 1))
            _, src1, dst1 = kv_rows(g, (t & (NSTR - 1)) ^ VX)
            c = t >> (NSTR.bit_length() - 1)
            return whole(k_hbm, k_v, slot, c, src0, dst0), whole(v_hbm, v_v, slot, c, src1, dst1)

        def edges_kv(piece):
            slot, src0, dst0 = kv_rows(piece >> 2, piece & 3)
            for e in range(2 * SHIFT):
                start((edge(k_hbm, k_v, slot, e, PER_HEAD, src0, dst0), edge(v_hbm, v_v, slot, e, PER_HEAD, src0, dst0)))

        def pair_woa(t):
            c, q = spread(t >> 1, PER_HEAD, WOA_NS), t & 1
            return tuple(whole(woa_hbm, wo_v, SEM_WOA, c, (q + k) * QR, (q + k) * QR) for k in (0, 2))

        def pair_wob(t):
            c, q = t >> 1, t & 1
            sem, first = SEM_WOB, 0
            for n in WOB[:-1]:
                first += n
                sem = sem + (c >= 4 * first).astype(jnp.int32)
            return tuple(whole(wob_hbm, wo_v, sem, c, (q + k) * QR, (4 + q + k) * QR) for k in (0, 2))

        seg_a = [(0, OFF_C, pair_qk), (OFF_C, OFF_QV, pair_c), (OFF_QV, OFF_KV, pair_qv),
                 (OFF_KV, OFF_KV + NSTR * KF, functools.partial(pair_kv, 0)),
                 (OFF_KV + NSTR * KF, END_A, functools.partial(pair_kv, 1))]
        seg_o = [(0, 2 * KF, pair_woa), (2 * KF, 4 * KF, pair_wob)]

        def issue(segments, g0, n, lo, hi):
            for s0, s1, pair in segments:
                if s1 <= lo or hi <= s0:
                    continue

                def one(t, carry, pair=pair):
                    start(pair(t))
                    return carry
                if isinstance(g0, int):
                    first, last = max(g0, s0), min(g0 + n, s1)
                else:
                    first = g0 if s0 <= lo else jnp.maximum(g0, s0)
                    last = g0 + n if hi <= s1 else jnp.minimum(g0 + n, s1)
                lax.fori_loop(first - s0, last - s0, one, 0)

        copy_xa = pltpu.make_async_copy(xa_hbm, xa_v, sems.at[SEM_QK])
        copy_xb = pltpu.make_async_copy(xb_hbm, xb_v, sems.at[SEM_QK])
        with scope("p0"):
            start((copy_xa, copy_xb))
            if SHIFT:
                def weight_edges(e, carry):
                    start((edge(wqa_hbm, wqa_v, SEM_QK, e, PER_W), edge(wuk_hbm, wuk_v, SEM_QK, e, PER_W)))
                    start((edge(c_hbm, c_v, SEM_C, e, PER_W), edge(c_hbm, c_v, SEM_C, e, PER_W, S, S)))
                    start((wqb_piece(PER_W - 1, e * (DESC // 16), DESC // 16), edge(wuv_hbm, wuv_v, SEM_QV, e, PER_W)))
                    return carry
                lax.fori_loop(0, 2, weight_edges, 0)
            issue(seg_a, 0, G1, 0, G1)
            if SHIFT:
                lax.fori_loop(0, LA, lambda t, c: (edges_kv(t), c)[1], 0)
            copy_xa.wait()
            copy_xb.wait()
            wait(wqa_v, SEM_QK)
            wait(wuk_v, SEM_QK)

        def rep_rows(x_v):
            return jnp.concatenate([jnp.broadcast_to(x_v[pl.ds(b, 1), :].astype(F32), (8, M)) for b in range(B)],
                                   axis=0).astype(BF16)

        def head_tiles(w_v, jj, cc):
            r0 = pl.multiple_of(cc * (128 * H // 2) + jj * 4, 4)
            w32 = w_v.bitcast(jnp.uint32).at[pl.ds(r0, 128 * H // 2 - 12)]
            tiles = []
            for u in range(4):
                w = w32[pl.ds(u, 128, stride=H // 2), :]
                tiles.append(pltpu.bitcast(w << 16, F32).astype(BF16))
                tiles.append(pltpu.bitcast(w & jnp.uint32(0xFFFF0000), F32).astype(BF16))
            return tiles

        sublane = lax.broadcasted_iota(jnp.int32, (8 * B, 128), 0) & 7
        zeros8 = tuple(jnp.zeros((8 * B, 128), F32) for _ in range(8))

        xa = rep_rows(xa_v)
        for cc in range(4):
            xa_s[cc] = xa[:, cc * 128:(cc + 1) * 128]

        def absorb(jj, carry):
            def q_step(cc, q):
                issue(seg_a, G1 + (jj * 8 + cc) * N1, N1, G1, G2)
                x = xa_s[cc]
                return tuple(q_r + _dot(x, w) for q_r, w in zip(q, head_tiles(wqa_v, jj, cc)))

            q = [q_r.astype(BF16) for q_r in lax.fori_loop(0, 4, q_step, zeros8)]

            def k_step(cc, carry):
                issue(seg_a, G1 + (jj * 8 + 4 + cc) * N1, N1, G1, G2)
                qa = None
                for r, w in enumerate(head_tiles(wuk_v, jj, cc)):
                    part = _dot_nt(q[r], w)
                    qa = part if r == 0 else jnp.where(sublane == r, part, qa)
                qabs_s[jj, cc] = qa
                return carry

            return lax.fori_loop(0, 4, k_step, carry)

        with scope("p1"):
            lax.fori_loop(0, H // 8, absorb, 0)

        wait(c_v, SEM_C)

        def latent(b, carry):
            rows_b = pl.ds(pl.multiple_of(b * 8, 8), 8)
            qa = jnp.concatenate([jnp.concatenate([qabs_s[jj, cc, rows_b, :] for cc in range(4)], axis=1)
                                  for jj in range(4)], axis=0).astype(BF16)

            def chunk(t):
                return c_v[pl.ds(pl.multiple_of(b * S + t * CH, CH), CH), :]

            def scores(t, m):
                issue(seg_a, G2 + (2 * b * NC + t) * N2, N2, G2, G3)
                s = _dot_nt(qa, chunk(t))
                s_s[t] = s
                return jnp.maximum(m, _fold(s, jnp.maximum))

            m = lax.fori_loop(0, NC, scores, jnp.full((H, 128), -jnp.inf, F32))
            m = jnp.max(m, axis=-1, keepdims=True)

            def values(t, carry):
                l, acc = carry
                issue(seg_a, G2 + ((2 * b + 1) * NC + t) * N2, N2, G2, G3)
                p = jnp.exp((s_s[t] - m) * scale)
                return l + _fold(p, jnp.add), acc + _dot(p.astype(BF16), chunk(t))

            l, acc = lax.fori_loop(0, NC, values, (jnp.zeros((H, 128), F32), jnp.zeros((H, C), F32)))
            ctx = acc / jnp.sum(l, axis=-1, keepdims=True)
            for jj in range(4):
                for cc in range(4):
                    ctx_s[jj, cc, rows_b, :] = ctx[8 * jj:8 * jj + 8, 128 * cc:128 * cc + 128]
            return carry

        with scope("p2"):
            lax.fori_loop(0, B, latent, 0)

        xb = rep_rows(xb_v)
        wait(wqb_v, SEM_QV)
        wait(wuv_v, SEM_QV)

        def project(jj, carry):
            def v_step(cc, o):
                j = jj * 4 + cc
                issue(seg_a, G3 + j * N3, N3, G3, G4)
                q = _dot(xb, wqb_v[:, pl.ds(pl.multiple_of(j * 2 * D, 2 * D), 2 * D)])
                for e in range(2):
                    for b in range(B):
                        qb_s[b * H + 2 * j + e] = q[8 * b:8 * b + 8, e * D:(e + 1) * D]
                ctx = ctx_s[jj, cc].astype(BF16)
                return tuple(o_r + _dot(ctx, w) for o_r, w in zip(o, head_tiles(wuv_v, jj, cc)))

            o = lax.fori_loop(0, 4, v_step, zeros8)
            for r in range(8):
                o_s[jj * 8 + r] = jnp.where(sublane == r, o[r], 0.0)
            return carry

        with scope("p3"):
            lax.fori_loop(0, H // 8, project, 0)

        def wo_edges(t, carry):
            e, q = t & 1, t >> 1
            start((edge(woa_hbm, wo_v, SEM_WOA, e, PER_HEAD, q * QR, q * QR),
                   edge(wob_hbm, wo_v, SEM_WOB + (len(WOB) - 1) * e, e, PER_HEAD, q * QR, (4 + q) * QR)))
            return carry

        def head(step, carry):
            g, j = step >> 2, step & 3
            slot, _, row0 = kv_rows(g, j)
            r = pl.ds(pl.multiple_of(row0, S), S)
            i = j * NSB + g
            q = qb_s[i].astype(BF16)

            def prefetch(part):
                ahead = step + LA
                if hsplit == 1:
                    k0, k1, o0, o1 = 0, KF, 0, N5
                else:
                    k0, k1 = ((0, KF // 2), (KF // 2, KF))[part]
                    o0, o1 = ((0, N5 // 2), (N5 // 2, N5))[part]

                @pl.when(ahead < NH)
                def _():
                    if part == 0:
                        edges_kv(ahead)
                    issue([(0, NSTR * KF, functools.partial(pair_kv, ahead >> 2))], (ahead & 3) * KF + k0, k1 - k0,
                          0, NSTR * KF)

                @pl.when(ahead >= NH)
                def _():
                    if SHIFT and part == 0:
                        lax.fori_loop(0, jnp.where(ahead == NH, 8, 0), wo_edges, 0)
                    issue(seg_o, (ahead - NH) * N5 + o0, o1 - o0, 0, G5)

            prefetch(0)

            @pl.when(j == 0)
            def _():
                block = pl.ds(pl.multiple_of(row0, NSTR * S), NSTR * S)
                wait(k_v.at[block], slot)
                wait(v_v.at[block], slot)

            s = _dot_nt(q, k_v[r, :])
            m = jnp.max(_fold(s, jnp.maximum), axis=-1, keepdims=True)
            p = jnp.exp((s - m) * scale)
            l = jnp.sum(_fold(p, jnp.add), axis=-1, keepdims=True)
            if hsplit == 2:
                prefetch(1)
            o = _dot(p.astype(BF16), v_v[r, :]) / l
            o_s[H + (i & (H - 1)), pl.ds(pl.multiple_of((j >> 1) * 8, 8), 8), :] = jnp.where(sublane[:8] == 0, o, 0.0)
            return carry

        def head_scoped(step, carry):
            with scope("step"):
                return head(step, carry)

        with scope("p4"):
            lax.fori_loop(0, NH, head_scoped, 0)

        half = SHIFT * (DESC // M // 2)

        def out_proj(side, carry):
            def group(p, acc):
                step = 8 * side + p
                if N6:
                    issue(seg_o, G5 + step * N6, N6, G5, G5 + 16 * N6)
                lhs = jnp.concatenate([o_s[side * H + q * 8 + p] for q in range(4)], axis=1).astype(BF16)

                first = 0
                for k, n in enumerate(WOB):
                    r0 = first * D + (half if first else 0)
                    r1 = min((first + n) * D + half, QR)

                    @pl.when(step == 8 + first)
                    def _():
                        for q in range(4):
                            wait(wo_v.at[pl.ds((4 + q) * QR + r0, r1 - r0)], SEM_WOB + k)
                    first += n
                w = jnp.concatenate([wo_v[pl.ds(pl.multiple_of((4 * side + q) * QR + p * D, D), D), :]
                                     for q in range(4)], axis=0)
                return acc + _dot(lhs, w)

            acc = lax.fori_loop(0, 8, group, jnp.zeros((8 * B, M), F32))
            for b in range(B):
                out_ref[pl.ds(b, 1), pl.ds(pl.multiple_of(side * M, M), M)] = jnp.sum(
                    acc[8 * b:8 * b + 8], axis=0, keepdims=True).astype(out_ref.dtype)
            return carry

        with scope("p5"):
            wait(wo_v.at[pl.ds(0, H * D)], SEM_WOA)
            lax.fori_loop(0, 2, out_proj, 0)

    def fn(A_x, A_c_kv, A_w_q, A_w_uk, A_w_uv, A_w_o, B_x, B_k_cache, B_v_cache, B_wq, B_wo):
        vm = pltpu.VMEM
        out = pl.pallas_call(
            _kernel,
            in_specs=[pl.BlockSpec(memory_space=pl.ANY)] * 11,
            out_specs=pl.BlockSpec(memory_space=pltpu.VMEM),
            out_shape=jax.ShapeDtypeStruct((B, 2 * M), A_x.dtype),
            scratch_shapes=[
                vm((B, M), BF16), vm((B, M), BF16),
                vm((B * S, C), BF16),
                vm((M * H, D), BF16), vm((C * H, D), BF16), vm((C * H, D), BF16),
                vm((M, H * D), BF16), vm((2 * H * D, M), BF16),
                vm((NSLOT * NSTR * S, D), BF16), vm((NSLOT * NSTR * S, D), BF16),
                vm((4, 8 * B, 128), BF16), vm((NH, 8, D), F32), vm((2 * H, 8 * B, D), F32),
                vm((4, 4, 8 * B, 128), F32), vm((4, 4, 8 * B, 128), F32), vm((S // CH, H, CH), F32),
                pltpu.SemaphoreType.DMA((NSEM,)),
            ],
            compiler_params=pltpu.CompilerParams(vmem_limit_bytes=vmem << 20, disable_bounds_checks=nobounds,
                                                 disable_semaphore_checks=nosem),
        )(A_x.reshape(B, M), A_c_kv.reshape(B * S, C),
          A_w_q.reshape(M * H, D), A_w_uk.reshape(C * H, D), A_w_uv.reshape(C * H, D), A_w_o.reshape(H * D, M),
          B_x.reshape(B, M), B_k_cache.reshape(NH * S, D), B_v_cache.reshape(NH * S, D), B_wq, B_wo)
        return out.reshape(B, 1, 2 * M)
    return fn


_impl = make(WOA_NS=4,WNS=4)


@jax.jit
def pallas_concat_heads__compressed_kv_cla__gqa_block_cached__decode_kernel(
        A_x, A_c_kv, A_w_q, A_w_uk, A_w_uv, A_w_o, B_x, B_k_cache, B_v_cache, B_wq, B_wo):
    return _impl(A_x, A_c_kv, A_w_q, A_w_uk, A_w_uv, A_w_o, B_x, B_k_cache, B_v_cache, B_wq, B_wo)
```

```python
import jax
import jax.numpy as jnp
import numpy as np
from jax import lax
from jax.experimental import pallas as pl
from jax.experimental.pallas import tpu as pltpu

F32 = jnp.float32
BF16 = jnp.bfloat16

B, H, S, D, M, C = 2, 32, 4096, 128, 512, 512
NH = B * H
SCALE = D ** -0.5

COPY = 16384
PER_HEAD = S * D // COPY
PER_W = M * H * D // COPY
STREAMS = 4
GROUPS = NH // STREAMS
SLOTS = 3
AHEAD = 6
CHUNK = 512
QUARTER = H * D // 4
WO_WAITS = (4, 2, 1, 1)

AT_C, AT_QV, AT_KV = PER_W, 2 * PER_W, 3 * PER_W
HEAD_END = AT_KV + AHEAD * PER_HEAD
N_ABSORB, N_LATENT, N_PROJECT = 4, 6, 5
AT_ABSORB = PER_W + 48
AT_LATENT = AT_ABSORB + 32 * N_ABSORB
AT_PROJECT = AT_LATENT + 2 * B * (S // CHUNK) * N_LATENT
AT_HEADS = AT_PROJECT + 16 * N_PROJECT
assert AT_LATENT >= AT_QV and AT_PROJECT >= AT_KV and AT_HEADS >= HEAD_END
N_WO = -(-PER_W // AHEAD)

SEM_QV, SEM_QK, SEM_C = 2, 3, 4
SEM_WOA, SEM_WOB = 1, 2
NSEM = SEM_WOB + len(WO_WAITS)
assert STREAMS < AHEAD <= 2 * STREAMS and (GROUPS - 1) % SLOTS == 0


def _dot(a, b):
    return jnp.dot(a, b, preferred_element_type=F32)


def _dot_nt(a, b):
    return lax.dot_general(a, b, (((1,), (1,)), ((), ())), preferred_element_type=F32)


def _fold(x, op):
    parts = [x[:, c:c + 128] for c in range(0, x.shape[1], 128)]
    while len(parts) > 1:
        parts = [op(parts[i], parts[i + 1]) for i in range(0, len(parts), 2)]
    return parts[0]


def _divmod(x, n):
    return x >> (n.bit_length() - 1), x & (n - 1)


def _spread(t, count, streams):
    position, stream = _divmod(t, streams)
    return stream * (count // streams) + position


def _body(xa_hbm, c_hbm, wq_hbm, wuk_hbm, wuv_hbm, woa_hbm, xb_hbm, k_hbm, v_hbm, wqb_hbm, wob_hbm,
          out_v, xa_v, xb_v, c_v, wq_v, wuk_v, wuv_v, wqb_v, wo_v, k_v, v_v,
          xa_s, qabs_s, s_s, ctx_s, qb_s, o_s, sems):
    def rows(src, dst, sem, c, src0=0, dst0=0):
        n = COPY // src.shape[1]
        return pltpu.make_async_copy(src.at[pl.ds(pl.multiple_of(src0 + c * n, n), n)],
                                     dst.at[pl.ds(pl.multiple_of(dst0 + c * n, n), n)], sems.at[sem])

    def start(pair):
        pair[0].start(priority=0)
        pair[1].start(priority=1)

    def wait(buf, sem):
        pltpu.make_async_copy(buf, buf, sems.at[sem]).wait()

    def pair_qk(t):
        c = _spread(t, PER_W, STREAMS)
        return rows(wq_hbm, wq_v, SEM_QK, c), rows(wuk_hbm, wuk_v, SEM_QK, c)

    def pair_c(t):
        c = _spread(t, PER_W, STREAMS)
        return rows(c_hbm, c_v, SEM_C, c), rows(c_hbm, c_v, SEM_C, c, S, S)

    def pair_qv(t):
        c = _spread(t, PER_W, STREAMS)
        r = pl.ds(pl.multiple_of((c >> 1) * 8, 8), 8)
        cols = pl.ds(pl.multiple_of((c & 1) * (COPY // 8), COPY // 8), COPY // 8)
        return (pltpu.make_async_copy(wqb_hbm.at[r, cols], wqb_v.at[r, cols], sems.at[SEM_QV]),
                rows(wuv_hbm, wuv_v, SEM_QV, c))

    def kv_place(g, j):
        slot = lax.rem(g, SLOTS)
        return slot, (j * GROUPS + g) * S, (slot * STREAMS + j) * S

    def pair_kv(g, t):
        c, j = _divmod(t, STREAMS)
        slot, src0, dst0 = kv_place(g, j)
        return rows(k_hbm, k_v, slot, c, src0, dst0), rows(v_hbm, v_v, slot, c, src0, dst0)

    def pair_woa(t):
        c, q = _spread(t >> 1, PER_HEAD, 2), t & 1
        return tuple(rows(woa_hbm, wo_v, SEM_WOA, c, (q + k) * QUARTER, (q + k) * QUARTER) for k in (0, 2))

    def pair_wob(t):
        c, q = t >> 1, t & 1
        sem, first = SEM_WOB, 0
        for n in WO_WAITS[:-1]:
            first += n
            sem = sem + (c >= first * (PER_HEAD // 8)).astype(jnp.int32)
        return tuple(rows(wob_hbm, wo_v, sem, c, (q + k) * QUARTER, (4 + q + k) * QUARTER) for k in (0, 2))

    per_group = STREAMS * PER_HEAD
    head_stream = [(0, AT_C, pair_qk), (AT_C, AT_QV, pair_c), (AT_QV, AT_KV, pair_qv),
                   (AT_KV, HEAD_END, lambda t: pair_kv(*_divmod(t, per_group)))]
    tail_stream = [(0, PER_W // 2, pair_woa), (PER_W // 2, PER_W, pair_wob)]

    def issue(stream, t0, n, lo, hi):
        for first, last, pair in stream:
            if last <= lo or hi <= first:
                continue

            def one(t, carry, pair=pair):
                start(pair(t))
                return carry

            if isinstance(t0, int):
                begin, end = max(t0, first), min(t0 + n, last)
            else:
                begin = t0 if first <= lo else jnp.maximum(t0, first)
                end = t0 + n if hi <= last else jnp.minimum(t0 + n, last)
            lax.fori_loop(begin - first, end - first, one, 0)

    def batch_rows(x_v):
        return jnp.concatenate(
            [jnp.broadcast_to(x_v[pl.ds(b, 1), :].astype(F32), (8, M)) for b in range(B)], axis=0).astype(BF16)

    def head_tiles(w_v, jj, cc):
        words = w_v.bitcast(jnp.uint32).at[pl.ds(pl.multiple_of(cc * (64 * H) + jj * 4, 4), 64 * H + 4)]
        tiles = []
        for u in range(4):
            w = words[pl.ds(u, 128, stride=H // 2), :]
            tiles.append(pltpu.bitcast(w << 16, F32).astype(BF16))
            tiles.append(pltpu.bitcast(w & np.uint32(0xFFFF0000), F32).astype(BF16))
        return tiles

    sublane = lax.broadcasted_iota(jnp.int32, (8 * B, D), 0) & 7
    zeros8 = tuple(jnp.zeros((8 * B, D), F32) for _ in range(8))

    copy_xa = pltpu.make_async_copy(xa_hbm, xa_v, sems.at[SEM_QK])
    copy_xb = pltpu.make_async_copy(xb_hbm, xb_v, sems.at[SEM_QK])
    start((copy_xa, copy_xb))
    issue(head_stream, 0, AT_ABSORB, 0, AT_ABSORB)
    copy_xa.wait()
    copy_xb.wait()
    wait(wq_v.at[pl.ds(0, M * H)], SEM_QK)
    wait(wuk_v.at[pl.ds(0, C * H)], SEM_QK)

    xa = batch_rows(xa_v)
    for cc in range(4):
        xa_s[cc] = xa[:, cc * 128:(cc + 1) * 128]

    def absorb(jj, carry):
        def q_step(cc, q):
            issue(head_stream, AT_ABSORB + (jj * 8 + cc) * N_ABSORB, N_ABSORB, AT_ABSORB, AT_LATENT)
            x = xa_s[cc]
            return tuple(q_r + _dot(x, w) for q_r, w in zip(q, head_tiles(wq_v, jj, cc)))

        q = [q_r.astype(BF16) for q_r in lax.fori_loop(0, 4, q_step, zeros8)]

        def k_step(cc, carry):
            issue(head_stream, AT_ABSORB + (jj * 8 + 4 + cc) * N_ABSORB, N_ABSORB, AT_ABSORB, AT_LATENT)
            qa = None
            for r, w in enumerate(head_tiles(wuk_v, jj, cc)):
                part = _dot_nt(q[r], w)
                qa = part if r == 0 else jnp.where(sublane == r, part, qa)
            qabs_s[jj, cc] = qa
            return carry

        return lax.fori_loop(0, 4, k_step, carry)

    lax.fori_loop(0, H // 8, absorb, 0)

    wait(c_v, SEM_C)
    chunks = S // CHUNK

    def latent(b, carry):
        rows_b = pl.ds(pl.multiple_of(b * 8, 8), 8)
        qa = jnp.concatenate(
            [jnp.concatenate([qabs_s[jj, cc, rows_b, :] for cc in range(4)], axis=1) for jj in range(4)],
            axis=0).astype(BF16)

        def chunk(t):
            return c_v[pl.ds(pl.multiple_of(b * S + t * CHUNK, CHUNK), CHUNK), :]

        def scores(t, m):
            issue(head_stream, AT_LATENT + (2 * b * chunks + t) * N_LATENT, N_LATENT, AT_LATENT, AT_PROJECT)
            s = _dot_nt(qa, chunk(t))
            s_s[t] = s
            return jnp.maximum(m, _fold(s, jnp.maximum))

        m = lax.fori_loop(0, chunks, scores, jnp.full((H, 128), -jnp.inf, F32))
        m = jnp.max(m, axis=-1, keepdims=True)

        def values(t, carry):
            l, acc = carry
            issue(head_stream, AT_LATENT + ((2 * b + 1) * chunks + t) * N_LATENT, N_LATENT, AT_LATENT, AT_PROJECT)
            p = jnp.exp((s_s[t] - m) * SCALE)
            return l + _fold(p, jnp.add), acc + _dot(p.astype(BF16), chunk(t))

        l, acc = lax.fori_loop(0, chunks, values, (jnp.zeros((H, 128), F32), jnp.zeros((H, C), F32)))
        ctx = acc / jnp.sum(l, axis=-1, keepdims=True)
        for jj in range(4):
            for cc in range(4):
                ctx_s[jj, cc, rows_b, :] = ctx[8 * jj:8 * jj + 8, 128 * cc:128 * cc + 128]
        return carry

    lax.fori_loop(0, B, latent, 0)

    wait(wqb_v, SEM_QV)
    wait(wuv_v.at[pl.ds(0, C * H)], SEM_QV)
    xb = batch_rows(xb_v)

    def project(jj, carry):
        def v_step(cc, o):
            j = jj * 4 + cc
            issue(head_stream, AT_PROJECT + j * N_PROJECT, N_PROJECT, AT_PROJECT, AT_HEADS)
            q = _dot(xb, wqb_v[:, pl.ds(pl.multiple_of(j * 2 * D, 2 * D), 2 * D)])
            for e in range(2):
                for b in range(B):
                    qb_s[b * H + 2 * j + e] = q[8 * b:8 * b + 8, e * D:(e + 1) * D]
            ctx = ctx_s[jj, cc].astype(BF16)
            return tuple(o_r + _dot(ctx, w) for o_r, w in zip(o, head_tiles(wuv_v, jj, cc)))

        o = lax.fori_loop(0, 4, v_step, zeros8)
        for r in range(8):
            o_s[jj * 8 + r] = jnp.where(sublane == r, o[r], 0.0)
        return carry

    lax.fori_loop(0, H // 8, project, 0)

    def head(step, carry):
        g, j = _divmod(step, STREAMS)
        slot, _, row0 = kv_place(g, j)
        r = pl.ds(pl.multiple_of(row0, S), S)
        i = j * GROUPS + g

        def prefetch(part):
            ahead = step + AHEAD

            @pl.when(ahead < NH)
            def _():
                n = PER_HEAD // 2
                g_ahead, j_ahead = _divmod(ahead, STREAMS)
                issue([(0, per_group, lambda t: pair_kv(g_ahead, t))], j_ahead * PER_HEAD + part * n, n, 0, per_group)

            @pl.when(ahead >= NH)
            def _():
                skip, n = ((0, N_WO // 2), (N_WO // 2, N_WO - N_WO // 2))[part]
                issue(tail_stream, (ahead - NH) * N_WO + skip, n, 0, AHEAD * N_WO)

        q = qb_s[i].astype(BF16)
        prefetch(0)

        @pl.when(j == 0)
        def _():
            group = pl.ds(pl.multiple_of(row0, STREAMS * S), STREAMS * S)
            wait(k_v.at[group], slot)
            wait(v_v.at[group], slot)

        s = _dot_nt(q, k_v[r, :])
        m = jnp.max(_fold(s, jnp.maximum), axis=-1, keepdims=True)
        p = jnp.exp((s - m) * SCALE)
        l = jnp.sum(_fold(p, jnp.add), axis=-1, keepdims=True)
        prefetch(1)
        o = _dot(p.astype(BF16), v_v[r, :]) / l
        b, h = _divmod(i, H)
        o_s[H + h, pl.ds(pl.multiple_of(b * 8, 8), 8), :] = jnp.where(sublane[:8] == 0, o, 0.0)
        return carry

    lax.fori_loop(0, NH, head, 0)

    def out_proj(side, carry):
        def step(p, acc):
            lhs = jnp.concatenate([o_s[side * H + q * 8 + p] for q in range(4)], axis=1).astype(BF16)
            first = 0
            for k, n in enumerate(WO_WAITS):
                @pl.when(8 * side + p == 8 + first)
                def _():
                    for q in range(4):
                        wait(wo_v.at[pl.ds((4 + q) * QUARTER + first * D, n * D)], SEM_WOB + k)
                first += n
            w = jnp.concatenate(
                [wo_v[pl.ds(pl.multiple_of((4 * side + q) * QUARTER + p * D, D), D), :] for q in range(4)], axis=0)
            return acc + _dot(lhs, w)

        acc = lax.fori_loop(0, 8, step, jnp.zeros((8 * B, M), F32))
        out = jnp.concatenate([jnp.sum(acc[8 * b:8 * b + 8], axis=0, keepdims=True) for b in range(B)], axis=0)
        out_v[:, pl.ds(pl.multiple_of(side * M, M), M)] = out.astype(out_v.dtype)
        return carry

    wait(wo_v.at[pl.ds(0, H * D)], SEM_WOA)
    lax.fori_loop(0, 2, out_proj, 0)


def _kernel(*refs):
    inputs, out_hbm, out_v, scratch, out_sem = refs[:11], refs[11], refs[12], refs[13:-1], refs[-1]
    copy_out = pltpu.make_async_copy(out_v, out_hbm, out_sem)

    def run(sems):
        _body(*inputs, out_v, *scratch, sems)
        copy_out.start()

    pl.run_scoped(run, pltpu.SemaphoreType.DMA((NSEM,)))
    copy_out.wait()


@jax.jit
def pallas_concat_heads__compressed_kv_cla__gqa_block_cached__decode_kernel(
    A_x: jax.Array,
    A_c_kv: jax.Array,
    A_w_q: jax.Array,
    A_w_uk: jax.Array,
    A_w_uv: jax.Array,
    A_w_o: jax.Array,
    B_x: jax.Array,
    B_k_cache: jax.Array,
    B_v_cache: jax.Array,
    B_wq: jax.Array,
    B_wo: jax.Array,
):
    assert A_x.shape == B_x.shape == (B, 1, M) and A_c_kv.shape == (B, S, C)
    assert A_w_q.shape == (M, H, D) and A_w_uk.shape == A_w_uv.shape == (C, H, D) and A_w_o.shape == (H, D, M)
    assert B_k_cache.shape == B_v_cache.shape == (B, H, S, D)
    assert B_wq.shape == (M, H * D) and B_wo.shape == (H * D, M)
    vmem = pltpu.VMEM
    out = pl.pallas_call(
        _kernel,
        in_specs=[pl.BlockSpec(memory_space=pl.ANY)] * 11,
        out_specs=pl.BlockSpec(memory_space=pl.ANY),
        out_shape=jax.ShapeDtypeStruct((B, 2 * M), A_x.dtype),
        scratch_shapes=[
            vmem((B, 2 * M), A_x.dtype),
            vmem((B, M), BF16), vmem((B, M), BF16),
            vmem((B * S, C), BF16),
            vmem((M * H + H, D), BF16), vmem((C * H + H, D), BF16), vmem((C * H + H, D), BF16),
            vmem((M, H * D), BF16),
            vmem((2 * H * D, M), BF16),
            vmem((SLOTS * STREAMS * S, D), BF16), vmem((SLOTS * STREAMS * S, D), BF16),
            vmem((4, 8 * B, 128), BF16),
            vmem((4, 4, 8 * B, 128), F32),
            vmem((S // CHUNK, H, CHUNK), F32),
            vmem((4, 4, 8 * B, 128), F32),
            vmem((NH, 8, D), F32),
            vmem((2 * H, 8 * B, D), F32),
            pltpu.SemaphoreType.DMA(()),
        ],
        compiler_params=pltpu.CompilerParams(vmem_limit_bytes=80 << 20),
    )(
        A_x.reshape(B, M), A_c_kv.reshape(B * S, C),
        A_w_q.reshape(M * H, D), A_w_uk.reshape(C * H, D), A_w_uv.reshape(C * H, D), A_w_o.reshape(H * D, M),
        B_x.reshape(B, M), B_k_cache.reshape(NH * S, D), B_v_cache.reshape(NH * S, D), B_wq, B_wo,
    )
    return out.reshape(B, 1, 2 * M)
```

```python
import jax
import jax.numpy as jnp
import numpy as np
from jax import lax
from jax.experimental import pallas as pl
from jax.experimental.pallas import tpu as pltpu

F32 = jnp.float32
BF16 = jnp.bfloat16

B, H, S, D, M, C = 2, 32, 4096, 128, 512, 512
NH = B * H
SCALE = D ** -0.5

COPY = 16384
PER_HEAD = S * D // COPY
PER_W = M * H * D // COPY
STREAMS = 4
GROUPS = NH // STREAMS
SLOTS = 4
AHEAD = 6
CHUNK = 512
QUARTER = H * D // 4
WO_WAITS = (4, 2, 1, 1)

AT_C, AT_QV, AT_KV = PER_W, 2 * PER_W, 3 * PER_W
HEAD_END = AT_KV + AHEAD * PER_HEAD
N_ABSORB, N_LATENT, N_PROJECT, N_REGROUP = 3, 5, 5, 6
AT_ABSORB = PER_W + 48
AT_LATENT = AT_ABSORB + 32 * N_ABSORB + 8 * N_REGROUP
AT_PROJECT = AT_LATENT + 2 * B * (S // CHUNK) * N_LATENT
AT_HEADS = AT_PROJECT + 16 * N_PROJECT + 4 * N_REGROUP
assert AT_LATENT >= AT_QV and AT_PROJECT >= AT_KV and AT_HEADS >= HEAD_END
N_WO = -(-PER_W // AHEAD)

SEM_QK, SEM_QV, SEM_C = 0, 3, 4
SEM_WOA, SEM_WOB = 1, 2
NSEM = SEM_WOB + len(WO_WAITS)
assert STREAMS < AHEAD < 2 * STREAMS and GROUPS % SLOTS == 0


def _dot(a, b):
    return jnp.dot(a, b, preferred_element_type=F32)


def _dot_nt(a, b):
    return lax.dot_general(a, b, (((1,), (1,)), ((), ())), preferred_element_type=F32)


def _fold(x, op):
    parts = [x[:, c:c + 128] for c in range(0, x.shape[1], 128)]
    while len(parts) > 1:
        parts = [op(parts[i], parts[i + 1]) for i in range(0, len(parts), 2)]
    return parts[0]


def _divmod(x, n):
    return x >> (n.bit_length() - 1), x & (n - 1)


def _spread(t, count, streams):
    position, stream = _divmod(t & (count - 1), streams)
    return stream * (count // streams) + position


def _body(xa_hbm, c_hbm, wq_hbm, wuk_hbm, wuv_hbm, woa_hbm, xb_hbm, k_hbm, v_hbm, wqb_hbm, wob_hbm,
          out_v, xa_v, xb_v, c_v, wq_v, wuk_v, wuv_v, wqb_v, wo_v, k_v, v_v,
          xa_s, words_s, qabs_s, s_s, ctx_s, qb_s, o_s, sems):
    def rows(src, dst, sem, c, src0=0, dst0=0):
        n = COPY // src.shape[1]
        return pltpu.make_async_copy(src.at[pl.ds(pl.multiple_of(src0 + c * n, n), n)],
                                     dst.at[pl.ds(pl.multiple_of(dst0 + c * n, n), n)], sems.at[sem])

    def start(pair):
        pair[0].start(priority=0)
        pair[1].start(priority=1)

    def wait(buf, sem):
        pltpu.make_async_copy(buf, buf, sems.at[sem]).wait()

    def pair_qk(t):
        c = _spread(t, PER_W, STREAMS)
        return rows(wq_hbm, wq_v, SEM_QK, c), rows(wuk_hbm, wuk_v, SEM_QK, c)

    def pair_c(t):
        c = _spread(t, PER_W, STREAMS)
        return rows(c_hbm, c_v, SEM_C, c), rows(c_hbm, c_v, SEM_C, c, S, S)

    def pair_qv(t):
        c = _spread(t, PER_W, STREAMS)
        r = pl.ds(pl.multiple_of((c >> 1) * 8, 8), 8)
        cols = pl.ds(pl.multiple_of((c & 1) * (COPY // 8), COPY // 8), COPY // 8)
        return (pltpu.make_async_copy(wqb_hbm.at[r, cols], wqb_v.at[r, cols], sems.at[SEM_QV]),
                rows(wuv_hbm, wuv_v, SEM_QV, c))

    per_group = STREAMS * PER_HEAD

    def kv_place(g, j):
        return (g + 1) & (SLOTS - 1), (j * GROUPS + g) * S, ((g & (SLOTS - 1)) * STREAMS + j) * S

    def pair_kv(g, t):
        c, j = _divmod(t & (per_group - 1), STREAMS)
        sem, src0, dst0 = kv_place(g & (GROUPS - 1), j)
        c = _spread(c, PER_HEAD, 2)
        return rows(k_hbm, k_v, sem, c, src0, dst0), rows(v_hbm, v_v, sem, c, src0, dst0)

    def pair_woa(t):
        c, q = _spread(t >> 1, PER_HEAD, 2), t & 1
        return tuple(rows(woa_hbm, wo_v, SEM_WOA, c, (q + k) * QUARTER, (q + k) * QUARTER) for k in (0, 2))

    def pair_wob(t):
        c, q = (t >> 1) & (PER_HEAD - 1), t & 1
        sem, first = SEM_WOB, 0
        for n in WO_WAITS[:-1]:
            first += n
            sem = sem + (c >= first * (PER_HEAD // 8)).astype(jnp.int32)
        return tuple(rows(wob_hbm, wo_v, sem, c, (q + k) * QUARTER, (4 + q + k) * QUARTER) for k in (0, 2))

    head_stream = [(0, AT_C, pair_qk), (AT_C, AT_QV, pair_c), (AT_QV, AT_KV, pair_qv),
                   (AT_KV, HEAD_END, lambda t: pair_kv(*_divmod(t, per_group)))]
    tail_stream = [(0, PER_W // 2, pair_woa), (PER_W // 2, PER_W, pair_wob)]

    def issue(stream, t0, n, lo, hi):
        for first, last, pair in stream:
            if last <= lo or hi <= first:
                continue

            def one(t, carry, pair=pair):
                start(pair(t))
                return carry

            if isinstance(t0, int):
                begin, end = max(t0, first), min(t0 + n, last)
            else:
                begin = t0 if first <= lo else jnp.maximum(t0, first)
                end = t0 + n if hi <= last else jnp.minimum(t0 + n, last)
            lax.fori_loop(begin - first, end - first, one, 0)

    def issue_weight_step(step, first, last, n, regrouping):
        def at(i):
            return first + i * n + jnp.minimum(i, regrouping) * N_REGROUP

        issue(head_stream, at(step), at(step + 1) - at(step), first, last)

    def batch_rows(x_v):
        return jnp.concatenate(
            [jnp.broadcast_to(x_v[pl.ds(b, 1), :].astype(F32), (8, M)) for b in range(B)], axis=0).astype(BF16)

    def head_tiles(w_v, words_s, jj, cc):
        @pl.when(jj == 0)
        def _():
            def regroup(t, carry):
                m0 = cc * 128 + t * 32
                w = pltpu.bitcast(w_v[pl.ds(pl.multiple_of(m0 * H, 32 * H), 32 * H), :], jnp.uint32)
                w = w.reshape(16, 4, 8, D)
                low = lax.broadcasted_iota(jnp.int32, (16, 8, D), 1) < 4
                for k in range(2):
                    even, odd = w[:, k], w[:, 2 + k]
                    dst = pl.ds(pl.multiple_of(m0 * 4, 128), 128)
                    words_s[2 * k, dst, :] = jnp.where(low, even, pltpu.roll(odd, 4, 1)).reshape(128, D)
                    words_s[2 * k + 1, dst, :] = jnp.where(low, pltpu.roll(even, 4, 1), odd).reshape(128, D)
                return carry

            lax.fori_loop(0, 4, regroup, 0)

        words = words_s.at[jj, pl.ds(pl.multiple_of(cc * 512, 512), 512 + 8)]
        tiles = []
        for u in range(4):
            w = words[pl.ds(u, 128, stride=4), :]
            tiles.append(pltpu.bitcast(w << 16, F32).astype(BF16))
            tiles.append(pltpu.bitcast(w & np.uint32(0xFFFF0000), F32).astype(BF16))
        return tiles

    sublane = lax.broadcasted_iota(jnp.int32, (8 * B, D), 0) & 7
    zeros8 = tuple(jnp.zeros((8 * B, D), F32) for _ in range(8))

    copy_xa = pltpu.make_async_copy(xa_hbm, xa_v, sems.at[SEM_QK])
    copy_xb = pltpu.make_async_copy(xb_hbm, xb_v, sems.at[SEM_QK])
    start((copy_xa, copy_xb))
    issue(head_stream, 0, AT_ABSORB, 0, AT_ABSORB)
    copy_xa.wait()
    copy_xb.wait()
    wait(wq_v, SEM_QK)
    wait(wuk_v, SEM_QK)

    xa = batch_rows(xa_v)
    for cc in range(4):
        xa_s[cc] = xa[:, cc * 128:(cc + 1) * 128]

    def absorb(jj, carry):
        def q_step(cc, q):
            issue_weight_step(jj * 8 + cc, AT_ABSORB, AT_LATENT, N_ABSORB, 8)
            x = xa_s[cc]
            return tuple(q_r + _dot(x, w) for q_r, w in zip(q, head_tiles(wq_v, words_s.at[0], jj, cc)))

        q = [q_r.astype(BF16) for q_r in lax.fori_loop(0, 4, q_step, zeros8)]

        def k_step(cc, carry):
            issue_weight_step(jj * 8 + 4 + cc, AT_ABSORB, AT_LATENT, N_ABSORB, 8)
            qa = None
            for r, w in enumerate(head_tiles(wuk_v, words_s.at[1], jj, cc)):
                part = _dot_nt(q[r], w)
                qa = part if r == 0 else jnp.where(sublane == r, part, qa)
            qabs_s[jj, cc] = qa
            return carry

        return lax.fori_loop(0, 4, k_step, carry)

    lax.fori_loop(0, H // 8, absorb, 0)

    wait(c_v, SEM_C)
    chunks = S // CHUNK

    def latent(b, carry):
        rows_b = pl.ds(pl.multiple_of(b * 8, 8), 8)
        qa = jnp.concatenate(
            [jnp.concatenate([qabs_s[jj, cc, rows_b, :] for cc in range(4)], axis=1) for jj in range(4)],
            axis=0).astype(BF16)

        def chunk(t):
            return c_v[pl.ds(pl.multiple_of(b * S + t * CHUNK, CHUNK), CHUNK), :]

        def scores(t, m):
            issue(head_stream, AT_LATENT + (2 * b * chunks + t) * N_LATENT, N_LATENT, AT_LATENT, AT_PROJECT)
            s = _dot_nt(qa, chunk(t))
            s_s[t] = s
            return jnp.maximum(m, _fold(s, jnp.maximum))

        m = lax.fori_loop(0, chunks, scores, jnp.full((H, 128), -jnp.inf, F32))
        m = jnp.max(m, axis=-1, keepdims=True)

        def values(t, carry):
            l, acc = carry
            issue(head_stream, AT_LATENT + ((2 * b + 1) * chunks + t) * N_LATENT, N_LATENT, AT_LATENT, AT_PROJECT)
            p = jnp.exp((s_s[t] - m) * SCALE)
            return l + _fold(p, jnp.add), acc + _dot(p.astype(BF16), chunk(t))

        l, acc = lax.fori_loop(0, chunks, values, (jnp.zeros((H, 128), F32), jnp.zeros((H, C), F32)))
        ctx = acc / jnp.sum(l, axis=-1, keepdims=True)
        for jj in range(4):
            for cc in range(4):
                ctx_s[jj, cc, rows_b, :] = ctx[8 * jj:8 * jj + 8, 128 * cc:128 * cc + 128]
        return carry

    lax.fori_loop(0, B, latent, 0)

    wait(wqb_v, SEM_QV)
    wait(wuv_v, SEM_QV)
    xb = batch_rows(xb_v)

    def project(jj, carry):
        def v_step(cc, o):
            j = jj * 4 + cc
            issue_weight_step(j, AT_PROJECT, AT_HEADS, N_PROJECT, 4)
            q = _dot(xb, wqb_v[:, pl.ds(pl.multiple_of(j * 2 * D, 2 * D), 2 * D)])
            for e in range(2):
                for b in range(B):
                    qb_s[b * H + 2 * j + e] = q[8 * b:8 * b + 8, e * D:(e + 1) * D]
            ctx = ctx_s[jj, cc].astype(BF16)
            return tuple(o_r + _dot(ctx, w) for o_r, w in zip(o, head_tiles(wuv_v, words_s.at[0], jj, cc)))

        o = lax.fori_loop(0, 4, v_step, zeros8)
        for r in range(8):
            o_s[jj * 8 + r] = jnp.where(sublane == r, o[r], 0.0)
        return carry

    lax.fori_loop(0, H // 8, project, 0)

    def head(step, carry):
        g, j = _divmod(step, STREAMS)
        sem, _, row0 = kv_place(g, j)
        r = pl.ds(pl.multiple_of(row0, S), S)
        i = j * GROUPS + g

        def prefetch(part):
            ahead = step + AHEAD

            @pl.when(ahead < NH)
            def _():
                n = PER_HEAD // 2
                g_ahead, j_ahead = _divmod(ahead, STREAMS)
                issue([(0, per_group, lambda t: pair_kv(g_ahead, t))], j_ahead * PER_HEAD + part * n, n, 0, per_group)

            @pl.when(ahead >= NH)
            def _():
                skip, n = ((0, N_WO // 2), (N_WO // 2, N_WO - N_WO // 2))[part]
                issue(tail_stream, (ahead - NH) * N_WO + skip, n, 0, AHEAD * N_WO)

        q = qb_s[i].astype(BF16)
        prefetch(0)

        @pl.when(j == 0)
        def _():
            group = pl.ds(pl.multiple_of(row0, STREAMS * S), STREAMS * S)
            wait(k_v.at[group], sem)
            wait(v_v.at[group], sem)

        s = _dot_nt(q, k_v[r, :])
        m = jnp.max(_fold(s, jnp.maximum), axis=-1, keepdims=True)
        p = jnp.exp((s - m) * SCALE)
        l = jnp.sum(_fold(p, jnp.add), axis=-1, keepdims=True)
        prefetch(1)
        o = _dot(p.astype(BF16), v_v[r, :]) / l
        b, h = _divmod(i, H)
        o_s[H + h, pl.ds(pl.multiple_of(b * 8, 8), 8), :] = jnp.where(sublane[:8] == 0, o, 0.0)
        return carry

    lax.fori_loop(0, NH, head, 0)

    def out_proj(side, carry):
        def step(p, acc):
            lhs = jnp.concatenate([o_s[side * H + q * 8 + p] for q in range(4)], axis=1).astype(BF16)
            first = 0
            for k, n in enumerate(WO_WAITS):
                @pl.when(8 * side + p == 8 + first)
                def _():
                    for q in range(4):
                        wait(wo_v.at[pl.ds((4 + q) * QUARTER + first * D, n * D)], SEM_WOB + k)
                first += n
            w = jnp.concatenate(
                [wo_v[pl.ds(pl.multiple_of((4 * side + q) * QUARTER + p * D, D), D), :] for q in range(4)], axis=0)
            return acc + _dot(lhs, w)

        acc = lax.fori_loop(0, 8, step, jnp.zeros((8 * B, M), F32))
        out = jnp.concatenate([jnp.sum(acc[8 * b:8 * b + 8], axis=0, keepdims=True) for b in range(B)], axis=0)
        out_v[:, pl.ds(pl.multiple_of(side * M, M), M)] = out.astype(out_v.dtype)
        return carry

    wait(wo_v.at[pl.ds(0, H * D)], SEM_WOA)
    lax.fori_loop(0, 2, out_proj, 0)


def _kernel(*refs):
    inputs, out_hbm, out_v, scratch, out_sem = refs[:11], refs[11], refs[12], refs[13:-1], refs[-1]
    copy_out = pltpu.make_async_copy(out_v, out_hbm, out_sem)

    def run(sems):
        _body(*inputs, out_v, *scratch, sems)
        copy_out.start()

    pl.run_scoped(run, pltpu.SemaphoreType.DMA((NSEM,)))
    copy_out.wait()


@jax.jit
def pallas_concat_heads__compressed_kv_cla__gqa_block_cached__decode_kernel(
    A_x: jax.Array,
    A_c_kv: jax.Array,
    A_w_q: jax.Array,
    A_w_uk: jax.Array,
    A_w_uv: jax.Array,
    A_w_o: jax.Array,
    B_x: jax.Array,
    B_k_cache: jax.Array,
    B_v_cache: jax.Array,
    B_wq: jax.Array,
    B_wo: jax.Array,
):
    assert A_x.shape == B_x.shape == (B, 1, M) and A_c_kv.shape == (B, S, C)
    assert A_w_q.shape == (M, H, D) and A_w_uk.shape == A_w_uv.shape == (C, H, D) and A_w_o.shape == (H, D, M)
    assert B_k_cache.shape == B_v_cache.shape == (B, H, S, D)
    assert B_wq.shape == (M, H * D) and B_wo.shape == (H * D, M)
    vmem = pltpu.VMEM
    out = pl.pallas_call(
        _kernel,
        in_specs=[pl.BlockSpec(memory_space=pl.ANY)] * 11,
        out_specs=pl.BlockSpec(memory_space=pl.ANY),
        out_shape=jax.ShapeDtypeStruct((B, 2 * M), A_x.dtype),
        scratch_shapes=[
            vmem((B, 2 * M), A_x.dtype),
            vmem((B, M), BF16), vmem((B, M), BF16),
            vmem((B * S, C), BF16),
            vmem((M * H, D), BF16), vmem((C * H, D), BF16), vmem((C * H, D), BF16),
            vmem((M, H * D), BF16),
            vmem((2 * H * D, M), BF16),
            vmem((SLOTS * STREAMS * S, D), BF16), vmem((SLOTS * STREAMS * S, D), BF16),
            vmem((4, 8 * B, 128), BF16),
            vmem((2, 4, 4 * M + 8, D), jnp.uint32),
            vmem((4, 4, 8 * B, 128), F32),
            vmem((S // CHUNK, H, CHUNK), F32),
            vmem((4, 4, 8 * B, 128), F32),
            vmem((NH, 8, D), F32),
            vmem((2 * H, 8 * B, D), F32),
            pltpu.SemaphoreType.DMA(()),
        ],
        compiler_params=pltpu.CompilerParams(vmem_limit_bytes=96 << 20),
    )(
        A_x.reshape(B, M), A_c_kv.reshape(B * S, C),
        A_w_q.reshape(M * H, D), A_w_uk.reshape(C * H, D), A_w_uv.reshape(C * H, D), A_w_o.reshape(H * D, M),
        B_x.reshape(B, M), B_k_cache.reshape(NH * S, D), B_v_cache.reshape(NH * S, D), B_wq, B_wo,
    )
    return out.reshape(B, 1, 2 * M)
```
